```python
import os as _os
_os.environ.setdefault("JAX_PLATFORMS", "cpu")
import jax
import jax.numpy as jnp

def _softmax(x, axis=-1):
    return jax.nn.softmax(x, axis=axis)
def _gelu(x):
    return jax.nn.gelu(x, approximate=True)
def _silu(x):
    return jax.nn.silu(x)
def _sigmoid(x):
    return jax.nn.sigmoid(x)
def _layernorm(x, axis=-1, eps=1e-5):
    m = jnp.mean(x, axis=axis, keepdims=True)
    v = jnp.var(x, axis=axis, keepdims=True)
    return (x - m) / jnp.sqrt(v + eps)
def _scatter_add(tgt, idx, src, axis=0):
    return tgt.at[idx].add(src)
def _segment_sum(src, seg, n):
    return jax.ops.segment_sum(src, seg, n)
class _Rng:
    def __init__(self, key):
        self._k = key
    def _next(self):
        self._k, sub = jax.random.split(self._k)
        return sub
    def normal(self, shape):
        return jax.random.normal(self._next(), shape, dtype=jnp.bfloat16)
    def randint(self, lo, hi, shape):
        return jax.random.randint(self._next(), shape, lo, hi, dtype=jnp.int32)
    def uniform(self, shape, lo=0.0, hi=1.0):
        return jax.random.uniform(self._next(), shape, jnp.bfloat16, lo, hi)
    def permutation(self, n):
        return jax.random.permutation(self._next(), n)


kernel_name = 'sequential_preLN__linear_kernel_hedgehog__dense_activation_squared_relu__prompt'

def setup_inputs():
    _rng = _Rng(jax.random.key(int.from_bytes(__import__("os").urandom(4), "little")))
    _w = (lambda a: (lambda t: t.astype(jnp.bfloat16) if jnp.issubdtype(t.dtype, jnp.floating) else t)(jnp.asarray(a)))
    def _A_setup():
        B, S, D, H = 1, 2048, 512, 32
        Dh = D // H
        return {
            "x": _w((lambda *s: _rng.normal(s) * 0.05)(B, S, D)),
            "wqkv": _w((lambda *s: _rng.normal(s) * 0.2)(D, 3 * D)),
            "w_phi": _w((lambda *s: _rng.normal(s) * 0.2)(H, Dh, Dh) * (Dh ** -0.5)),
            "wo": _w((lambda *s: _rng.normal(s) * 0.05)(D, D)),
        }
    _A_in = _A_setup()

    def _B_setup():
        B, S, D, F = 1, 2048, 512, 1792
        return {
            "x": _w((lambda *s: _rng.normal(s) * 0.05)(B, S, D)),
            "w1": _w((lambda *s: _rng.normal(s) * 0.05)(D, F)),
            "b1": _w((lambda *s: _rng.normal(s) * 0.05)(F)),
            "w2": _w((lambda *s: _rng.normal(s) * 0.05)(F, D)),
            "b2": _w((lambda *s: _rng.normal(s) * 0.05)(D)),
        }
    _B_in = _B_setup()

    return {
        "A_x": _A_in["x"],
        "A_wqkv": _A_in["wqkv"],
        "A_w_phi": _A_in["w_phi"],
        "A_wo": _A_in["wo"],
        "B_x": _B_in["x"],
        "B_w1": _B_in["w1"],
        "B_b1": _B_in["b1"],
        "B_w2": _B_in["w2"],
        "B_b2": _B_in["b2"],
    }

def reference(A_x, A_wqkv, A_w_phi, A_wo, B_x, B_w1, B_b1, B_w2, B_b2):
    def _A_ref(x, wqkv, w_phi, wo):
        B, S, D = x.shape
        H = 32; Dh = D // H
        qkv = (lambda x, *d: x.transpose(*d))((x @ wqkv).reshape(B, S, 3, H, Dh), 2, 0, 3, 1, 4)
        q, k, v = qkv[0], qkv[1], qkv[2]
        pq = jnp.einsum("bhsd,hdf->bhsf", q, w_phi)
        pk = jnp.einsum("bhsd,hdf->bhsf", k, w_phi)
        phi_q = jnp.concatenate([_softmax(pq, axis=-1), _softmax(-pq, axis=-1)], axis=-1)
        phi_k = jnp.concatenate([_softmax(pk, axis=-1), _softmax(-pk, axis=-1)], axis=-1)
        kv = jnp.einsum("bhsf,bhsd->bhfd", phi_k, v)
        z  = jnp.einsum("bhsf->bhf", phi_k)
        num = jnp.einsum("bhqf,bhfd->bhqd", phi_q, kv)
        den = jnp.einsum("bhqf,bhf->bhq", phi_q, z)[..., None] + 1e-6
        o = num / den
        return (lambda x, *d: x.transpose(*d))(o, 0, 2, 1, 3).reshape(B, S, D) @ wo

    def _B_ref(x, w1, b1, w2, b2):
        h = jnp.einsum("bsd,df->bsf", x, w1) + b1
        zero = jnp.zeros_like(h)
        r = jnp.where(h > zero, h, zero)
        h = r * r
        out = jnp.einsum("bsf,fd->bsd", h, w2) + b2
        return out

    x = A_x
    h = x + _A_ref(_layernorm(x, axis=-1), A_wqkv, A_w_phi, A_wo)
    h2 = h + _B_ref(_layernorm(h, axis=-1), B_w1, B_b1, B_w2, B_b2)
    return h2
```

```python
import numpy as np
import jax
import jax.numpy as jnp
from jax import lax
import jax.experimental.pallas as pl
import jax.experimental.pallas.tpu as pltpu

S, D, H, DH, F = 2048, 512, 32, 16, 1792
T1 = 256
T2 = 256
FC = 256
ORD = "a"
ORD1 = "b"
XB = "0.1.2.3"
WA = 2
SPLITW = 0
SC = 0
DS = "p.k.x0|v.x1|x2.x3|q.o.b.c.1.2"
PRE = 0
LOG2E = 1.4426950408889634
BF = jnp.bfloat16
F32 = jnp.float32
NT = (((1,), (1,)), ((), ()))


def _dot(a, b):
    return jnp.dot(a, b, preferred_element_type=F32)


def _dot_nt(a, b):
    return lax.dot_general(a, b, NT, preferred_element_type=F32)


def _ln(x):
    m = jnp.mean(x, axis=-1, keepdims=True)
    c = x - m
    v = jnp.mean(c * c, axis=-1, keepdims=True)
    return c * lax.rsqrt(v + 1e-5)


def _iota(shape, d):
    return lax.broadcasted_iota(jnp.int32, shape, d)


def _red(x, op):
    y = x[:, 0]
    for j in range(1, 8):
        y = op(y, x[:, j])
    y = op(y, pltpu.roll(y, 4, 1))
    return y[:, None]


def _feat(pT, T):
    p = pT.reshape(8, 8, 8, T)
    mx = _red(p, jnp.maximum)
    mn = _red(p, jnp.minimum)
    ep = jnp.exp2(p - mx)
    en = jnp.exp2(mn - p)
    rp = 1.0 / _red(ep, jnp.add)
    rn = 1.0 / _red(en, jnp.add)
    return ep, en, rp, rn


def _kernel(x_hbm, wqkv_hbm, wphi_hbm, wo_hbm, w1_hbm, b1_hbm, w2_hbm, b2_hbm,
            o_hbm,
            x_v, xn_v, wq_v, wk_v, wv_v, wphi_v, wo_v, w1_v, b1_v, w2_v, b2_v,
            wqT_v, wkvT_v, o_v, xsem, wsem, osem):
    n1 = S // T1
    n2 = S // T2

    def cp(src, dst, i):
        return pltpu.make_async_copy(src, dst, wsem.at[i])

    c_phi = cp(wphi_hbm, wphi_v, 0)
    c_wk = cp(wqkv_hbm.at[:, D:2 * D], wk_v, 1)
    c_wv = cp(wqkv_hbm.at[:, 2 * D:3 * D], wv_v, 2)
    c_wq = cp(wqkv_hbm.at[:, 0:D], wq_v, 3)
    c_wo = cp(wo_hbm, wo_v, 4)
    c_w1 = cp(w1_hbm, w1_v, 5)
    c_w2 = cp(w2_hbm, w2_v, 6)
    c_b1 = cp(b1_hbm, b1_v, 7)
    c_b2 = cp(b2_hbm, b2_v, 8)
    xb = [int(b) * T1 for b in XB.split(".")] + [S]
    c_x = [pltpu.make_async_copy(x_hbm.at[xb[j]:xb[j + 1]], x_v.at[xb[j]:xb[j + 1]], xsem.at[j])
           for j in range(len(xb) - 1)]
    c_o = [pltpu.make_async_copy(o_v.at[i * T2:(i + 1) * T2], o_hbm.at[i * T2:(i + 1) * T2], osem.at[i])
           for i in range(n2)]

    def issue(stage):
        for k in DS.split("|")[stage].split("."):
            if k == "": continue
            {"p": c_phi, "k": c_wk, "v": c_wv, "q": c_wq, "o": c_wo, "1": c_w1, "2": c_w2, "b": c_b1, "c": c_b2}[k].start() \
                if not k.startswith("x") else c_x[int(k[1:])].start()

    issue(0)
    c_phi.wait()
    wp = wphi_v[...]
    sel = (_iota((32, 512), 0) == _iota((32, 512), 1) // 16).astype(BF)
    xw = _dot(wp, sel)
    xw = jnp.where(_iota((256, 512), 0) // 16 == _iota((256, 512), 1) % 16, xw, 0.0).astype(BF)
    rsel = ((_iota((128, 256), 0) % 64) // 4 == _iota((128, 256), 1) % 16).astype(BF)
    bd = _dot(rsel, xw)
    ci = _iota((128, 512), 0)
    hi = _iota((128, 512), 1) // 16
    bd = jnp.where(((ci // 64) * 4 + ci % 4) == hi % 8, bd, 0.0).astype(BF)

    def fold(w_ref, dst, row0):
        for g in range(4):
            r = _dot_nt(bd[:, g * 128:(g + 1) * 128], w_ref[:, g * 128:(g + 1) * 128])
            dst[row0 + g * 128:row0 + (g + 1) * 128, :] = (r * LOG2E).astype(BF)

    c_wk.wait()
    issue(1)
    fold(wk_v, wkvT_v, 0)

    def ln_tile(i):
        xs = x_v[i * T1:(i + 1) * T1, :].astype(F32)
        xn_v[i * T1:(i + 1) * T1, :] = _ln(xs).astype(BF)

    c_x[0].wait()
    issue(2)
    ln_tile(0)
    c_wv.wait()
    wkvT_v[D:2 * D, :] = wv_v[...].astype(F32).T.astype(BF)

    s1 = {}
    acc = {}

    def MM(i):
        s1['pv', i] = _dot_nt(wkvT_v[...], xn_v[i * T1:(i + 1) * T1, :])

    def SM(i):
        pv = s1.pop(('pv', i))
        ep, en, rp, rn = _feat(pv[0:D], T1)
        php = ep * rp
        phn = en * rn
        s1['vT', i] = pv[D:2 * D].astype(BF)
        zt, ph = [], []
        for g in range(8):
            phi = jnp.concatenate([php[g].reshape(64, T1), phn[g].reshape(64, T1)], axis=0)
            zz = phi[:, 0:128]
            for j in range(1, T1 // 128):
                zz = zz + phi[:, j * 128:(j + 1) * 128]
            zt.append(zz)
            ph.append(phi.astype(BF))
        s1['phi', i] = ph
        acc['z'] = zt if i == 0 else [a + b for a, b in zip(acc['z'], zt)]

    def KV(i):
        vT, ph = s1.pop(('vT', i)), s1.pop(('phi', i))
        kvt = [_dot_nt(vT[g * 64:(g + 1) * 64], ph[g]) for g in range(8)]
        acc['kv'] = kvt if i == 0 else [a + b for a, b in zip(acc['kv'], kvt)]

    def LN(i):
        ln_tile(i)

    def XW(i):
        if i < n1 and i * T1 in xb:
            c_x[xb.index(i * T1)].wait()

    def FOLDQ():
        fold(wq_v, wqT_v, 0)

    fin = {}

    def WAITALL():
        c_wq.wait()
        if not SPLITW: WAIT2()

    def WAIT2():
        c_wo.wait(); c_b1.wait(); c_b2.wait(); c_w1.wait(); c_w2.wait()

    def FIN():
        kmask = (_iota((64, 128), 0) // 16) == (_iota((64, 128), 1) % 4)
        fin['kvT'] = [jnp.where(kmask, a, 0.0).astype(BF) for a in acc['kv']]
        fin['zb'] = [jnp.broadcast_to(jnp.sum(a, axis=1, keepdims=True), (128, 128)) for a in acc['z']]

    def WAITW():
        if SPLITW: WAIT2()
        b1 = b1_v[...].astype(F32)
        b2 = b2_v[...].astype(F32)
        fin['b1'] = jnp.concatenate([b1[j:j + 1, :] for j in range(F // 128)], axis=1)
        fin['b2'] = jnp.concatenate([b2[j:j + 1, :] for j in range(D // 128)], axis=1)

    T = T2
    st = {}

    def A1(i):
        st['pq', i] = _dot_nt(wqT_v[...], xn_v[i * T:(i + 1) * T, :])

    def A2(i):
        zb = fin['zb']
        ep, en, rp, rn = _feat(st.pop(('pq', i)), T)
        zp = jnp.stack([jnp.concatenate([z[0:64]] * (T // 128), axis=1).reshape(8, 8, T) for z in zb])
        zn = jnp.stack([jnp.concatenate([z[64:128]] * (T // 128), axis=1).reshape(8, 8, T) for z in zb])
        den = rp * _red(ep * zp, jnp.add) + rn * _red(en * zn, jnp.add) + 1e-6
        rd = 1.0 / den
        php = ep * (rp * rd)
        phn = en * (rn * rd)
        st['phi', i] = [jnp.concatenate([php[g].reshape(64, T), phn[g].reshape(64, T)], axis=0).astype(BF)
                        for g in range(8)]

    def A3(i):
        phi = st.pop(('phi', i))
        oT = jnp.concatenate([_dot(fin['kvT'][g], phi[g]) for g in range(8)], axis=0)
        st['o', i] = oT.T.astype(BF)

    def A4(i):
        h = x_v[i * T:(i + 1) * T, :].astype(F32) + _dot(st.pop(('o', i)), wo_v[...])
        st['h', i] = h
        st['hn', i] = _ln(h).astype(BF)

    def B1(i, c):
        a = _dot(st['hn', i], w1_v[:, c * FC:(c + 1) * FC]) + fin['b1'][:, c * FC:(c + 1) * FC]
        a = jnp.maximum(a, 0.0)
        st['a', i, c] = (a * a).astype(BF)

    def B2(i):
        a = jnp.concatenate([st.pop(('a', i, c)) for c in range(F // FC)], axis=1)
        st.pop(('hn', i))
        y = _dot(a, w2_v[...]) + fin['b2'] + st.pop(('h', i))
        o_v[i * T:(i + 1) * T, :] = y.astype(BF)
        c_o[i].start()

    issue(3)
    sc = jax.named_scope('p1') if SC else None
    if sc: sc.__enter__()
    if ORD1 == "a":
        XW(1); MM(0); LN(1)
        for i in range(n1):
            if i == n1 - WA: WAITALL()
            XW(i + 2)
            if i + 1 < n1: MM(i + 1)
            else: FOLDQ()
            SM(i)
            if i + 2 < n1: LN(i + 2)
            KV(i)
        A1(0); WAITW()
    elif ORD1 == "b":
        XW(1); MM(0); LN(1)
        for i in range(n1):
            SM(i)
            if i == n1 - WA: WAITALL()
            XW(i + 2)
            if i + 1 < n1: MM(i + 1)
            else: FOLDQ()
            if i + 2 < n1: LN(i + 2)
            KV(i)
        A1(0); WAITW()
    elif ORD1 == "c":
        XW(1); MM(0); LN(1)
        for i in range(n1):
            if i == n1 - WA: WAITALL()
            XW(i + 2)
            if i + 1 < n1: MM(i + 1)
            else: FOLDQ()
            if i + 2 < n1: LN(i + 2)
            if i > 0: KV(i - 1)
            SM(i)
        A1(0)
        KV(n1 - 1); WAITW()
    FIN()
    if sc: sc.__exit__(None, None, None)
    sc = jax.named_scope('p2') if SC else None
    if sc: sc.__enter__()

    nc = F // FC
    A1(1) if PRE else None
    A2(0); A3(0); A4(0)
    for i in range(n2):
        nxt = i + 1 < n2
        if ORD == "a":
            q1, q2 = (2 * nc) // 7, (4 * nc) // 7
            if nxt and not (PRE and i == 0): A1(i + 1)
            for c in range(0, q1): B1(i, c)
            if nxt: A2(i + 1)
            for c in range(q1, q2): B1(i, c)
            if nxt: A3(i + 1)
            for c in range(q2, nc): B1(i, c)
            if nxt: A4(i + 1)
            B2(i)
        else:
            for c in range(nc): B1(i, c)
            B2(i)
            if nxt:
                A1(i + 1); A2(i + 1); A3(i + 1); A4(i + 1)
    if sc: sc.__exit__(None, None, None)
    for c in c_o:
        c.wait()


@jax.jit
def pallas_sequential_preLN__linear_kernel_hedgehog__dense_activation_squared_relu__prompt_kernel(
        A_x, A_wqkv, A_w_phi, A_wo, B_x, B_w1, B_b1, B_w2, B_b2):
    del B_x
    hbm = pl.BlockSpec(memory_space=pl.ANY)
    out = pl.pallas_call(
        _kernel,
        in_specs=[hbm] * 8,
        out_specs=hbm,
        out_shape=jax.ShapeDtypeStruct((S, D), BF),
        scratch_shapes=[
            pltpu.VMEM((S, D), BF),
            pltpu.VMEM((S, D), BF),
            pltpu.VMEM((D, D), BF),
            pltpu.VMEM((D, D), BF),
            pltpu.VMEM((D, D), BF),
            pltpu.VMEM((DH * DH, H), BF),
            pltpu.VMEM((D, D), BF),
            pltpu.VMEM((D, F), BF),
            pltpu.VMEM((F // 128, 128), BF),
            pltpu.VMEM((F, D), BF),
            pltpu.VMEM((D // 128, 128), BF),
            pltpu.VMEM((D, D), BF),
            pltpu.VMEM((2 * D, D), BF),
            pltpu.VMEM((S, D), BF),
            pltpu.SemaphoreType.DMA((S // T1,)),
            pltpu.SemaphoreType.DMA((9,)),
            pltpu.SemaphoreType.DMA((S // T2,)),
        ],
        compiler_params=pltpu.CompilerParams(vmem_limit_bytes=100 * 1024 * 1024),
    )(A_x.reshape(S, D), A_wqkv, jnp.transpose(A_w_phi, (1, 2, 0)).reshape(DH * DH, H), A_wo, B_w1,
      B_b1.reshape(F // 128, 128), B_w2, B_b2.reshape(D // 128, 128))
    return out.reshape(1, S, D)
```

```python
import jax
import jax.numpy as jnp
from jax import lax
import jax.experimental.pallas as pl
import jax.experimental.pallas.tpu as pltpu

S, D, H, DH, F = 2048, 512, 32, 16, 1792
T = 256
NTILE = S // T
FC = 256
LOG2E = 1.4426950408889634
BF = jnp.bfloat16
F32 = jnp.float32
NT = (((1,), (1,)), ((), ()))
SCHED = (
    "I.p.k.x0 J.v.x1 W.p J.x2.x3 BD W.k.x0 J.q.o FK LN.0 MK.0 W.v.x1 J.b.c.1.2 LN.1 TV MV.0 SM.0 MK.1 "
    "SM.1 MV.1 W.x2.x3 LN.2 LN.4 KV.0 LN.3 KV.1 MK.4 MK.2 MK.3 MV.2 LN.5 MV.3 SM.2 MK.5 SM.4 SM.3 "
    "MV.4 KV.2 LN.6 KV.3 MV.5 MK.6 SM.5 LN.7 KV.5 MV.6 SM.6 KV.6 MK.7 KV.4 W.q.o.b.c.1.2 FQ SM.7 FZ "
    "MV.7 KV.7 FV A1.0 A2.0 A1.1 BI A3.0 A1.2 A4.0 A1.3 B1.0.0 B1.0.1 B1.0.6 A2.1 A3.1 B1.0.3 A1.4 "
    "B1.0.4 B1.0.2 B1.0.5 A4.1 B2.0.1 B1.1.1 B1.1.0 A2.2 B1.1.2 B1.1.4 B1.1.3 A3.2 B1.1.5 B1.1.6 A4.2 "
    "B2.1.1 B1.2.0 A1.5 A2.3 B1.2.3 B1.2.1 B1.2.2 B1.2.5 B1.2.4 A3.3 B1.2.6 A4.3 A2.4 B2.2.1 B1.3.0 "
    "B1.3.1 A1.6 B1.3.2 B1.3.3 A3.4 B1.3.4 B1.3.5 B1.3.6 A4.4 B2.3.1 B1.4.0 A1.7 B1.4.1 A2.5 B1.4.2 "
    "A3.5 B1.4.3 B1.4.4 B1.4.5 B1.4.6 A4.5 B2.4.1 B1.5.0 B1.5.1 A2.6 B1.5.2 B1.5.3 A3.6 B1.5.4 B1.5.5 "
    "B1.5.6 A4.6 B2.5.1 B1.6.2 B1.6.0 B1.6.1 A2.7 B1.6.3 A3.7 B1.6.4 B1.6.5 B1.6.6 A4.7 B2.6.1 B1.7.0 "
    "B1.7.1 B1.7.5 B1.7.2 B1.7.3 B1.7.4 B1.7.6 B2.7.4 "
)


def _dot(a, b):
    return jnp.dot(a, b, preferred_element_type=F32)


def _dot_nt(a, b):
    return lax.dot_general(a, b, NT, preferred_element_type=F32)


def _ln(x):
    m = jnp.mean(x, axis=-1, keepdims=True)
    c = x - m
    v = jnp.mean(c * c, axis=-1, keepdims=True)
    return c * lax.rsqrt(v + 1e-5)


def _iota(shape, d):
    return lax.broadcasted_iota(jnp.int32, shape, d)


def _red(x, op):
    y = x[:, 0]
    for j in range(1, 8):
        y = op(y, x[:, j])
    y = op(y, pltpu.roll(y, 4, 1))
    return y[:, None]


def _feat(pT):
    p = pT.reshape(8, 8, 8, T)
    mx = _red(p, jnp.maximum)
    mn = _red(p, jnp.minimum)
    ep = jnp.exp2(p - mx)
    en = jnp.exp2(mn - p)
    rp = 1.0 / _red(ep, jnp.add)
    rn = 1.0 / _red(en, jnp.add)
    return ep, en, rp, rn


def _kernel(x_hbm, wqkv_hbm, wphi_hbm, wo_hbm, w1_hbm, b1_hbm, w2_hbm, b2_hbm,
            o_hbm,
            x_v, xn_v, wq_v, wk_v, wv_v, wphi_v, wo_v, w1_v, b1_v, w2_v, b2_v,
            wqT_v, wkT_v, wvT_v, o_v, isem, osem):
    cin = {}

    def mk(name, src, dst):
        cin[name] = pltpu.make_async_copy(src, dst, isem.at[len(cin)])

    mk("p", wphi_hbm, wphi_v)
    mk("k", wqkv_hbm.at[:, D:2 * D], wk_v)
    mk("v", wqkv_hbm.at[:, 2 * D:3 * D], wv_v)
    mk("q", wqkv_hbm.at[:, 0:D], wq_v)
    mk("o", wo_hbm, wo_v)
    mk("1", w1_hbm, w1_v)
    mk("2", w2_hbm, w2_v)
    mk("b", b1_hbm, b1_v)
    mk("c", b2_hbm, b2_v)
    for (a, b) in ((0, 1), (1, 2), (2, 3), (3, NTILE)):
        mk(f"x{a}", x_hbm.at[a * T:b * T], x_v.at[a * T:b * T])
    cout = []

    st = {}
    rows = lambda i: slice(i * T, (i + 1) * T)

    def I(*names):
        for n in names:
            cin[n].start()

    def J(*names):
        for n in names:
            cin[n].start(priority=1)

    def W(*names):
        for n in names:
            cin[n].wait()

    def BD():
        wp = wphi_v[...]
        sel = (_iota((32, 512), 0) == _iota((32, 512), 1) // 16).astype(BF)
        xw = _dot(wp, sel)
        xw = jnp.where(_iota((256, 512), 0) // 16 == _iota((256, 512), 1) % 16, xw, 0.0).astype(BF)
        rsel = ((_iota((128, 256), 0) % 64) // 4 == _iota((128, 256), 1) % 16).astype(BF)
        bd = _dot(rsel, xw)
        ci = _iota((128, 512), 0)
        hi = _iota((128, 512), 1) // 16
        st["bd"] = jnp.where(((ci // 64) * 4 + ci % 4) == hi % 8, bd, 0.0).astype(BF)

    def fold(w_ref, dst):
        bd = st["bd"]
        for g in range(4):
            r = _dot_nt(bd[:, g * 128:(g + 1) * 128], w_ref[:, g * 128:(g + 1) * 128])
            dst[g * 128:(g + 1) * 128, :] = (r * LOG2E).astype(BF)

    def FK():
        fold(wk_v, wkT_v)

    def FQ():
        fold(wq_v, wqT_v)

    def TV():
        wvT_v[...] = wv_v[...].astype(F32).T.astype(BF)

    def LN(i):
        xn_v[rows(i), :] = _ln(x_v[rows(i), :].astype(F32)).astype(BF)

    def MK(i):
        st["pk", i] = _dot_nt(wkT_v[...], xn_v[rows(i), :])

    def MV(i):
        st["vT", i] = _dot_nt(wvT_v[...], xn_v[rows(i), :]).astype(BF)

    def SM(i):
        ep, en, rp, rn = _feat(st.pop(("pk", i)))
        php = ep * rp
        phn = en * rn
        zt, ph = [], []
        for g in range(8):
            phi = jnp.concatenate([php[g].reshape(64, T), phn[g].reshape(64, T)], axis=0)
            zz = phi[:, 0:128]
            for j in range(1, T // 128):
                zz = zz + phi[:, j * 128:(j + 1) * 128]
            zt.append(zz)
            ph.append(phi.astype(BF))
        st["phik", i] = ph
        st["z"] = zt if "z" not in st else [a + b for a, b in zip(st["z"], zt)]

    def KV(i):
        vT, ph = st.pop(("vT", i)), st.pop(("phik", i))
        kvt = [_dot_nt(vT[g * 64:(g + 1) * 64], ph[g]) for g in range(8)]
        st["kv"] = kvt if "kv" not in st else [a + b for a, b in zip(st["kv"], kvt)]

    def FZ():
        st["zb"] = [jnp.broadcast_to(jnp.sum(a, axis=1, keepdims=True), (128, 128)) for a in st["z"]]

    def FV():
        kmask = (_iota((64, 128), 0) // 16) == (_iota((64, 128), 1) % 4)
        st["kvT"] = [jnp.where(kmask, a, 0.0).astype(BF) for a in st["kv"]]

    def BI():
        b1 = b1_v[...].astype(F32)
        b2 = b2_v[...].astype(F32)
        st["b1"] = jnp.concatenate([b1[j:j + 1, :] for j in range(F // 128)], axis=1)
        st["b2"] = jnp.concatenate([b2[j:j + 1, :] for j in range(D // 128)], axis=1)

    def A1(i):
        st["pq", i] = _dot_nt(wqT_v[...], xn_v[rows(i), :])

    def A2(i):
        zb = st["zb"]
        ep, en, rp, rn = _feat(st.pop(("pq", i)))
        zp = jnp.stack([jnp.concatenate([z[0:64]] * (T // 128), axis=1).reshape(8, 8, T) for z in zb])
        zn = jnp.stack([jnp.concatenate([z[64:128]] * (T // 128), axis=1).reshape(8, 8, T) for z in zb])
        den = rp * _red(ep * zp, jnp.add) + rn * _red(en * zn, jnp.add) + 1e-6
        rd = 1.0 / den
        php = ep * (rp * rd)
        phn = en * (rn * rd)
        st["phiq", i] = [jnp.concatenate([php[g].reshape(64, T), phn[g].reshape(64, T)], axis=0).astype(BF)
                         for g in range(8)]

    def A3(i):
        phi = st.pop(("phiq", i))
        oT = jnp.concatenate([_dot(st["kvT"][g], phi[g]) for g in range(8)], axis=0)
        st["o", i] = oT.T.astype(BF)

    def A4(i):
        h = x_v[rows(i), :].astype(F32) + _dot(st.pop(("o", i)), wo_v[...])
        st["h", i] = h
        st["hn", i] = _ln(h).astype(BF)

    def B1(i, c):
        a = _dot(st["hn", i], w1_v[:, c * FC:(c + 1) * FC]) + st["b1"][:, c * FC:(c + 1) * FC]
        a = jnp.maximum(a, 0.0)
        st["a", i, c] = (a * a).astype(BF)

    def B2(i, nsplit=1):
        a = jnp.concatenate([st.pop(("a", i, c)) for c in range(F // FC)], axis=1)
        st.pop(("hn", i))
        h = st.pop(("h", i))
        R = T // nsplit
        for s in range(nsplit):
            y = _dot(a[s * R:(s + 1) * R], w2_v[...]) + st["b2"] + h[s * R:(s + 1) * R]
            r0 = i * T + s * R
            o_v[r0:r0 + R, :] = y.astype(BF)
            c = pltpu.make_async_copy(o_v.at[r0:r0 + R], o_hbm.at[r0:r0 + R], osem.at[len(cout)])
            c.start()
            cout.append(c)

    ops = dict(I=I, J=J, W=W, BD=BD, FK=FK, FQ=FQ, TV=TV, LN=LN, MK=MK, MV=MV, SM=SM, KV=KV, FZ=FZ, FV=FV,
               BI=BI, A1=A1, A2=A2, A3=A3, A4=A4, B1=B1, B2=B2)
    for tok in SCHED.split():
        name, *args = tok.split(".")
        if name not in ("I", "J", "W"):
            args = [int(a) for a in args]
        ops[name](*args)
    for c in cout:
        c.wait()


@jax.jit
def pallas_sequential_preLN__linear_kernel_hedgehog__dense_activation_squared_relu__prompt_kernel(
        A_x, A_wqkv, A_w_phi, A_wo, B_x, B_w1, B_b1, B_w2, B_b2):
    del B_x
    hbm = pl.BlockSpec(memory_space=pl.ANY)
    out = pl.pallas_call(
        _kernel,
        in_specs=[hbm] * 8,
        out_specs=hbm,
        out_shape=jax.ShapeDtypeStruct((S, D), BF),
        scratch_shapes=[
            pltpu.VMEM((S, D), BF),
            pltpu.VMEM((S, D), BF),
            pltpu.VMEM((D, D), BF),
            pltpu.VMEM((D, D), BF),
            pltpu.VMEM((D, D), BF),
            pltpu.VMEM((DH * DH, H), BF),
            pltpu.VMEM((D, D), BF),
            pltpu.VMEM((D, F), BF),
            pltpu.VMEM((F // 128, 128), BF),
            pltpu.VMEM((F, D), BF),
            pltpu.VMEM((D // 128, 128), BF),
            pltpu.VMEM((D, D), BF),
            pltpu.VMEM((D, D), BF),
            pltpu.VMEM((D, D), BF),
            pltpu.VMEM((S, D), BF),
            pltpu.SemaphoreType.DMA((13,)),
            pltpu.SemaphoreType.DMA((NTILE + 8,)),
        ],
        compiler_params=pltpu.CompilerParams(vmem_limit_bytes=100 * 1024 * 1024),
    )(A_x.reshape(S, D), A_wqkv, jnp.transpose(A_w_phi, (1, 2, 0)).reshape(DH * DH, H), A_wo, B_w1,
      B_b1.reshape(F // 128, 128), B_w2, B_b2.reshape(D // 128, 128))
    return out.reshape(1, S, D)
```
